```python
import os as _os
_os.environ.setdefault("JAX_PLATFORMS", "cpu")
import jax
import jax.numpy as jnp

def _softmax(x, axis=-1):
    return jax.nn.softmax(x, axis=axis)
def _gelu(x):
    return jax.nn.gelu(x, approximate=True)
def _silu(x):
    return jax.nn.silu(x)
def _sigmoid(x):
    return jax.nn.sigmoid(x)
def _layernorm(x, axis=-1, eps=1e-5):
    m = jnp.mean(x, axis=axis, keepdims=True)
    v = jnp.var(x, axis=axis, keepdims=True)
    return (x - m) / jnp.sqrt(v + eps)
def _scatter_add(tgt, idx, src, axis=0):
    return tgt.at[idx].add(src)
def _segment_sum(src, seg, n):
    return jax.ops.segment_sum(src, seg, n)
class _Rng:
    def __init__(self, key):
        self._k = key
    def _next(self):
        self._k, sub = jax.random.split(self._k)
        return sub
    def normal(self, shape):
        return jax.random.normal(self._next(), shape, dtype=jnp.bfloat16)
    def randint(self, lo, hi, shape):
        return jax.random.randint(self._next(), shape, lo, hi, dtype=jnp.int32)
    def uniform(self, shape, lo=0.0, hi=1.0):
        return jax.random.uniform(self._next(), shape, jnp.bfloat16, lo, hi)
    def permutation(self, n):
        return jax.random.permutation(self._next(), n)


kernel_name = 'parallel_sum__mha_block_cached__dense_activation_mish__decode'

def setup_inputs():
    _rng = _Rng(jax.random.key(int.from_bytes(__import__("os").urandom(4), "little")))
    _w = (lambda a: (lambda t: t.astype(jnp.bfloat16) if jnp.issubdtype(t.dtype, jnp.floating) else t)(jnp.asarray(a)))
    def _A_setup():
        B, Sq, D = 1, 1, 448
        H, Sk, Dh = 16, 16384, 256
        return {
            "x": _w((lambda *s: _rng.normal(s) * 0.05)(B, Sq, D)),
            "k_cache": _w((lambda *s: _rng.normal(s) * 1.6)(B, H, Sk, Dh)),
            "v_cache": _w((lambda *s: _rng.normal(s) * 0.8)(B, H, Sk, Dh)),
            "wq": _w((lambda *s: _rng.normal(s) * 1.6)(D, H * Dh) * (D ** -0.5)),
            "wo": _w((lambda *s: _rng.normal(s) * 0.8)(H * Dh, D) * ((H * Dh) ** -0.5)),
        }
    _A_in = _A_setup()

    def _B_setup():
        B, S, D, F = 1, 1, 448, 1792
        return {
            "x": _w((lambda *s: _rng.normal(s) * 0.05)(B, S, D)),
            "w1": _w((lambda *s: _rng.normal(s) * 0.8)(D, F) * (D ** -0.5)),
            "b1": _w((lambda *s: _rng.normal(s) * 0.05)(F)),
            "w2": _w((lambda *s: _rng.normal(s) * 0.05)(F, D) * (F ** -0.5)),
        }
    _B_in = _B_setup()

    return {
        "A_x": _A_in["x"],
        "A_k_cache": _A_in["k_cache"],
        "A_v_cache": _A_in["v_cache"],
        "A_wq": _A_in["wq"],
        "A_wo": _A_in["wo"],
        "B_x": _B_in["x"],
        "B_w1": _B_in["w1"],
        "B_b1": _B_in["b1"],
        "B_w2": _B_in["w2"],
    }

def reference(A_x, A_k_cache, A_v_cache, A_wq, A_wo, B_x, B_w1, B_b1, B_w2):
    def _A_ref(x, k_cache, v_cache, wq, wo):
        B, Sq, D = x.shape
        H, Dh = 16, 256
        q = (lambda x, *d: x.transpose(*d))((x @ wq).reshape(B, Sq, H, Dh), 0, 2, 1, 3)
        scores = jnp.einsum("bhqd,bhkd->bhqk", q, k_cache) * (Dh ** -0.5)
        p = _softmax(scores, axis=-1)
        o = jnp.einsum("bhqk,bhkd->bhqd", p, v_cache)
        return (lambda x, *d: x.transpose(*d))(o, 0, 2, 1, 3).reshape(B, Sq, H * Dh) @ wo

    def _B_ref(x, w1, b1, w2):
        h = jnp.einsum("bsd,df->bsf", x, w1) + b1
        sp = jnp.log1p(jnp.exp(-jnp.abs(h))) + jnp.where(h > 0, h, jnp.zeros_like(h))
        act = h * jnp.tanh(sp)
        return jnp.einsum("bsf,fd->bsd", act, w2)

    x = A_x
    xn = _layernorm(x, axis=-1)
    return x + _A_ref(xn, A_k_cache, A_v_cache, A_wq, A_wo) + _B_ref(xn, B_w1, B_b1, B_w2)
```

```python
import jax
import jax.numpy as jnp
from jax import lax
from jax.experimental import pallas as pl
from jax.experimental.pallas import tpu as pltpu

bf = jnp.bfloat16
f32 = jnp.float32
D, H, SK, DH, F = 448, 16, 16384, 256, 1792
T = 128
NG = SK // T
NT = (((1,), (1,)), ((), ()))


def make(nbuf=8, lag=4, hq=8, nobc=True, nosc=False, unroll_issue=False, compute=True):
    assert lag < nbuf

    def kernel(x_hbm, k_hbm, v_hbm, wq_hbm, wot_hbm, w1_hbm, b1_hbm, w2t_hbm, o_hbm,
               x_v, b1_v, wq_v, wot_v, w1_v, w2t_v, buf, s_v, q_v, ob_v, out_v,
               gsem, wsem):
        X, B1, WQ, W1, W2, OUT, WO = 0, 1, 2, 3, 4, 5, 6

        def issue_cache(src, g, slot):
            r0 = pl.multiple_of(g * T, T)
            def one(h, _):
                for half in range(2):
                    for qn in range(2):
                        hh = h + hq * qn if hq == 8 else (h // hq) * 2 * hq + h % hq + hq * qn
                        pltpu.make_async_copy(
                            src.at[0, hh, pl.ds(r0 + half * 64, 64), :],
                            buf.at[slot, hh, pl.ds(half * 64, 64), :],
                            gsem.at[slot]).start(priority=qn)
            if unroll_issue:
                for h in range(8): one(h, None)
            else:
                lax.fori_loop(0, 8, one, None)

        def wait_group(slot):
            pltpu.make_async_copy(buf.at[slot], buf.at[slot], gsem.at[slot]).wait()

        def issue_wide(src, dst, sem, lo, hi):
            def one(i, _):
                rg = (i % 2) * 14 + i // 2
                for half in range(2):
                    for qn in range(2):
                        r = pl.multiple_of((rg + 28 * qn) * 8, 8)
                        pltpu.make_async_copy(
                            src.at[pl.ds(r, 8), pl.ds(half * 2048, 2048)],
                            dst.at[pl.ds(r, 8), pl.ds(half * 2048, 2048)],
                            sem).start(priority=qn)
            lax.fori_loop(lo, hi, one, None)

        def issue_ffn(lo, hi):
            def one(i, _):
                rg = (i % 2) * 28 + (i // 2) * 2
                for half in range(2):
                    r = pl.multiple_of((rg + half) * 8, 8)
                    pltpu.make_async_copy(w1_hbm.at[pl.ds(r, 8)], w1_v.at[pl.ds(r, 8)], wsem.at[W1]).start(priority=0)
                    pltpu.make_async_copy(w2t_hbm.at[pl.ds(r, 8)], w2t_v.at[pl.ds(r, 8)], wsem.at[W2]).start(priority=1)
            lax.fori_loop(lo, hi, one, None)

        def issue_wo(nb):
            n = 8 if nb < 3 else 4
            def one(i, _):
                for half in range(2):
                    for qn in range(2):
                        r = pl.multiple_of(nb * 128 + (i + n * qn) * 8, 8)
                        pltpu.make_async_copy(
                            wot_hbm.at[pl.ds(r, 8), pl.ds(half * 2048, 2048)],
                            wot_v.at[pl.ds(r, 8), pl.ds(half * 2048, 2048)],
                            wsem.at[WO + nb]).start(priority=qn)
            lax.fori_loop(0, n, one, None)

        def wait_all(ref, sem):
            pltpu.make_async_copy(ref, ref, sem).wait()

        cx = pltpu.make_async_copy(x_hbm, x_v, wsem.at[X]); cx.start()
        cb = pltpu.make_async_copy(b1_hbm, b1_v, wsem.at[B1]); cb.start(priority=1)
        issue_wide(wq_hbm, wq_v, wsem.at[WQ], 0, 28)
        issue_ffn(0, 28)
        cx.wait(); cb.wait()
        x = x_v[0].astype(f32)
        mu = jnp.mean(x, axis=-1, keepdims=True)
        xc = x - mu
        var = jnp.mean(xc * xc, axis=-1, keepdims=True)
        xn = jnp.broadcast_to(xc / jnp.sqrt(var + 1e-5), (8, D)).astype(bf)

        row = lax.broadcasted_iota(jnp.int32, (8, DH), 0)
        wait_all(wq_v, wsem.at[WQ])

        def qstep(i, _):
            @pl.when(i < lag)
            def _(): issue_cache(k_hbm, i, i)
            for j in range(4):
                h = i * 4 + j
                c0 = pl.multiple_of(h * DH, DH)
                q = jnp.dot(xn, wq_v[:, pl.ds(c0, DH)], preferred_element_type=f32)
                q = q.astype(bf).astype(f32) * (DH ** -0.5)
                q_v[h] = jnp.where(row == h % 8, q, 0.0)
        lax.fori_loop(0, 4, qstep, None)
        for g in range(4, lag):
            issue_cache(k_hbm, g, g)

        wait_all(w1_v, wsem.at[W1])
        hpre = jnp.dot(xn, w1_v[...], preferred_element_type=f32)
        b1 = b1_v[...].astype(f32)
        bias = jnp.concatenate([jnp.broadcast_to(b1[j:j + 1], (8, 128)) for j in range(F // 128)], axis=1)
        hh = hpre + bias
        sp = jnp.log1p(jnp.exp(-jnp.abs(hh))) + jnp.maximum(hh, 0.0)
        act = (hh * jnp.tanh(sp)).astype(bf)
        wait_all(w2t_v, wsem.at[W2])
        base = lax.dot_general(act, w2t_v[...], NT, preferred_element_type=f32) + x

        def kstep(g, m):
            slot = g % nbuf
            nxt = g + lag
            @pl.when(nxt < NG)
            def _(): issue_cache(k_hbm, nxt, nxt % nbuf)
            @pl.when(nxt >= NG)
            def _(): issue_cache(v_hbm, nxt - NG, nxt % nbuf)
            wait_group(slot)
            if not compute: return m
            parts = []
            for a in range(2):
                s = None
                for j in range(8):
                    h = a * 8 + j
                    d = lax.dot_general(q_v[h].astype(bf), buf[slot, h], NT, preferred_element_type=f32)
                    s = d if s is None else s + d
                parts.append(s)
            s = jnp.concatenate(parts, axis=0)
            s_v[g] = s
            return jnp.maximum(m, s)
        m = lax.fori_loop(0, NG, kstep, jnp.full((H, T), -jnp.inf, f32))
        m = jnp.broadcast_to(jnp.max(m, axis=-1, keepdims=True), (H, T))

        row8 = lax.broadcasted_iota(jnp.int32, (8, T), 0)

        def vstep(g, carry):
            l, acc0, acc1 = carry
            slot = (g + NG) % nbuf
            nxt = g + lag
            @pl.when(nxt < NG)
            def _(): issue_cache(v_hbm, nxt, (nxt + NG) % nbuf)
            for nb in range(min(4, lag)):
                @pl.when(nxt == NG + nb)
                def _(): issue_wo(nb)
            wait_group(slot)
            if not compute: return carry
            p = jnp.exp(s_v[g] - m)
            accs = [acc0, acc1]
            for a in range(2):
                pa = p[a * 8:(a + 1) * 8]
                for j in range(8):
                    ph = jnp.where(row8 == j, pa, 0.0).astype(bf)
                    accs[a] = accs[a] + jnp.dot(ph, buf[slot, a * 8 + j], preferred_element_type=f32)
            return l + p, accs[0], accs[1]
        z = jnp.zeros((8, DH), f32)
        l, acc0, acc1 = lax.fori_loop(0, NG, vstep, (jnp.zeros((H, T), f32), z, z))
        for nb in range(lag, 4):
            issue_wo(nb)
        l = jnp.sum(l, axis=-1, keepdims=True)
        o = jnp.concatenate([acc0, acc1], axis=0) / l
        ob = jnp.concatenate([jnp.broadcast_to(o[h:h + 1], (8, DH)) for h in range(H)], axis=1).astype(bf)
        ys = []
        for nb in range(4):
            n = 128 if nb < 3 else 64
            blk = wot_v.at[pl.ds(nb * 128, n)]
            wait_all(blk, wsem.at[WO + nb])
            ys.append(lax.dot_general(ob, blk[...], NT, preferred_element_type=f32))
        y = jnp.concatenate(ys, axis=1) + base
        out_v[0] = y[0:1].astype(bf)
        co = pltpu.make_async_copy(out_v, o_hbm, wsem.at[OUT]); co.start(); co.wait()

    def f(A_x, A_k, A_v, A_wq, A_wo, B_x, B_w1, B_b1, B_w2):
        hbm = pl.BlockSpec(memory_space=pltpu.HBM)
        return pl.pallas_call(
            kernel, out_shape=jax.ShapeDtypeStruct((1, 1, D), bf),
            in_specs=[hbm] * 8, out_specs=hbm,
            scratch_shapes=[
                pltpu.VMEM((1, 1, D), bf), pltpu.VMEM((F // 128, 128), bf),
                pltpu.VMEM((D, H * DH), bf), pltpu.VMEM((D, H * DH), bf),
                pltpu.VMEM((D, F), bf), pltpu.VMEM((D, F), bf),
                pltpu.VMEM((nbuf, H, T, DH), bf), pltpu.VMEM((NG, H, T), f32),
                pltpu.VMEM((H, 8, DH), f32), pltpu.VMEM((8, H * DH), f32), pltpu.VMEM((1, 1, D), bf),
                pltpu.SemaphoreType.DMA((nbuf,)), pltpu.SemaphoreType.DMA((10,))],
            compiler_params=pltpu.CompilerParams(vmem_limit_bytes=64 << 20, disable_bounds_checks=nobc,
                                                 disable_semaphore_checks=nosc),
        )(A_x, A_k, A_v, A_wq, A_wo.T, B_w1, B_b1.reshape(F // 128, 128), B_w2.T)
    return f


@jax.jit
def pallas_parallel_sum__mha_block_cached__dense_activation_mish__decode_kernel(
    A_x, A_k_cache, A_v_cache, A_wq, A_wo, B_x, B_w1, B_b1, B_w2):
    return make(lag=3, nbuf=4)(A_x, A_k_cache, A_v_cache, A_wq, A_wo, B_x, B_w1, B_b1, B_w2)
```

```python
import jax
import jax.numpy as jnp
from jax import lax
from jax.experimental import pallas as pl
from jax.experimental.pallas import tpu as pltpu

bf = jnp.bfloat16
f32 = jnp.float32
D, H, SK, DH, F = 448, 16, 16384, 256, 1792
T = 128
NG = SK // T
NT = (((1,), (1,)), ((), ()))


def make(nbuf=8, lag=4, hq=8, nobc=True, nosc=False, unroll_issue=False, compute=True):
    assert lag < nbuf

    def kernel(x_hbm, k_hbm, v_hbm, wq_hbm, wot_hbm, w1_hbm, b1_hbm, w2t_hbm, o_hbm,
               x_v, b1_v, wq_v, wot_v, w1_v, w2t_v, buf, s_v, q_v, ob_v, out_v,
               gsem, wsem):
        X, B1, WQ, W1, W2, OUT, WO = 0, 1, 2, 3, 4, 5, 6

        def issue_cache(src, g, slot):
            r0 = pl.multiple_of(g * T, T)
            def one(i, _):
                half = i // 4
                ro = pl.multiple_of(half * 64, 64)
                for j in range(4):
                    hh = (i % 4) * 4 + j
                    pltpu.make_async_copy(
                        src.at[0, hh, pl.ds(r0 + ro, 64), :],
                        buf.at[slot, hh, pl.ds(ro, 64), :],
                        gsem.at[slot]).start(priority=j % 2)
            lax.fori_loop(0, 8, one, None)

        def wait_group(slot):
            pltpu.make_async_copy(buf.at[slot], buf.at[slot], gsem.at[slot]).wait()

        def issue_wide(src, dst, sem, lo, hi):
            def one(i, _):
                rg = (i % 2) * 14 + i // 2
                for half in range(2):
                    for qn in range(2):
                        r = pl.multiple_of((rg + 28 * qn) * 8, 8)
                        pltpu.make_async_copy(
                            src.at[pl.ds(r, 8), pl.ds(half * 2048, 2048)],
                            dst.at[pl.ds(r, 8), pl.ds(half * 2048, 2048)],
                            sem).start(priority=qn)
            lax.fori_loop(lo, hi, one, None)

        def issue_ffn(lo, hi):
            def one(i, _):
                rg = (i % 2) * 28 + (i // 2) * 2
                for half in range(2):
                    r = pl.multiple_of((rg + half) * 8, 8)
                    pltpu.make_async_copy(w1_hbm.at[pl.ds(r, 8)], w1_v.at[pl.ds(r, 8)], wsem.at[W1]).start(priority=0)
                    pltpu.make_async_copy(w2t_hbm.at[pl.ds(r, 8)], w2t_v.at[pl.ds(r, 8)], wsem.at[W2]).start(priority=1)
            lax.fori_loop(lo, hi, one, None)

        def issue_wo(nb):
            n = 8 if nb < 3 else 4
            def one(i, _):
                for half in range(2):
                    for qn in range(2):
                        r = pl.multiple_of(nb * 128 + (i + n * qn) * 8, 8)
                        pltpu.make_async_copy(
                            wot_hbm.at[pl.ds(r, 8), pl.ds(half * 2048, 2048)],
                            wot_v.at[pl.ds(r, 8), pl.ds(half * 2048, 2048)],
                            wsem.at[WO + nb]).start(priority=qn)
            lax.fori_loop(0, n, one, None)

        def wait_all(ref, sem):
            pltpu.make_async_copy(ref, ref, sem).wait()

        cx = pltpu.make_async_copy(x_hbm, x_v, wsem.at[X]); cx.start()
        cb = pltpu.make_async_copy(b1_hbm, b1_v, wsem.at[B1]); cb.start(priority=1)
        issue_wide(wq_hbm, wq_v, wsem.at[WQ], 0, 28)
        issue_ffn(0, 28)
        cx.wait(); cb.wait()
        x = x_v[0].astype(f32)
        mu = jnp.mean(x, axis=-1, keepdims=True)
        xc = x - mu
        var = jnp.mean(xc * xc, axis=-1, keepdims=True)
        xn = jnp.broadcast_to(xc / jnp.sqrt(var + 1e-5), (8, D)).astype(bf)

        row = lax.broadcasted_iota(jnp.int32, (8, DH), 0)
        wait_all(wq_v, wsem.at[WQ])

        def qstep(i, _):
            @pl.when(i < lag)
            def _(): issue_cache(k_hbm, i, i)
            for j in range(4):
                h = i * 4 + j
                c0 = pl.multiple_of(h * DH, DH)
                q = jnp.dot(xn, wq_v[:, pl.ds(c0, DH)], preferred_element_type=f32)
                q = q.astype(bf).astype(f32) * (DH ** -0.5)
                q_v[h] = jnp.where(row == h % 8, q, 0.0)
        lax.fori_loop(0, 4, qstep, None)
        for g in range(4, lag):
            issue_cache(k_hbm, g, g)

        wait_all(w1_v, wsem.at[W1])
        hpre = jnp.dot(xn, w1_v[...], preferred_element_type=f32)
        b1 = b1_v[...].astype(f32)
        bias = jnp.concatenate([jnp.broadcast_to(b1[j:j + 1], (8, 128)) for j in range(F // 128)], axis=1)
        hh = hpre + bias
        sp = jnp.log1p(jnp.exp(-jnp.abs(hh))) + jnp.maximum(hh, 0.0)
        act = (hh * jnp.tanh(sp)).astype(bf)
        wait_all(w2t_v, wsem.at[W2])
        base = lax.dot_general(act, w2t_v[...], NT, preferred_element_type=f32) + x

        def kstep(g, m):
            slot = g % nbuf
            nxt = g + lag
            @pl.when(nxt < NG)
            def _(): issue_cache(k_hbm, nxt, nxt % nbuf)
            @pl.when(nxt >= NG)
            def _(): issue_cache(v_hbm, nxt - NG, nxt % nbuf)
            wait_group(slot)
            if not compute: return m
            parts = []
            for a in range(2):
                s = None
                for j in range(8):
                    h = a * 8 + j
                    d = lax.dot_general(q_v[h].astype(bf), buf[slot, h], NT, preferred_element_type=f32)
                    s = d if s is None else s + d
                parts.append(s)
            s = jnp.concatenate(parts, axis=0)
            s_v[g] = s
            return jnp.maximum(m, s)
        m = lax.fori_loop(0, NG, kstep, jnp.full((H, T), -jnp.inf, f32))
        m = jnp.broadcast_to(jnp.max(m, axis=-1, keepdims=True), (H, T))

        row8 = lax.broadcasted_iota(jnp.int32, (8, T), 0)

        def vstep(g, carry):
            l, acc0, acc1 = carry
            slot = (g + NG) % nbuf
            nxt = g + lag
            @pl.when(nxt < NG)
            def _(): issue_cache(v_hbm, nxt, (nxt + NG) % nbuf)
            for nb in range(min(4, lag)):
                @pl.when(nxt == NG + nb)
                def _(): issue_wo(nb)
            wait_group(slot)
            if not compute: return carry
            p = jnp.exp(s_v[g] - m)
            accs = [acc0, acc1]
            for a in range(2):
                pa = p[a * 8:(a + 1) * 8]
                for j in range(8):
                    ph = jnp.where(row8 == j, pa, 0.0).astype(bf)
                    accs[a] = accs[a] + jnp.dot(ph, buf[slot, a * 8 + j], preferred_element_type=f32)
            return l + p, accs[0], accs[1]
        z = jnp.zeros((8, DH), f32)
        l, acc0, acc1 = lax.fori_loop(0, NG, vstep, (jnp.zeros((H, T), f32), z, z))
        for nb in range(lag, 4):
            issue_wo(nb)
        l = jnp.sum(l, axis=-1, keepdims=True)
        o = jnp.concatenate([acc0, acc1], axis=0) / l
        ob = jnp.concatenate([jnp.broadcast_to(o[h:h + 1], (8, DH)) for h in range(H)], axis=1).astype(bf)
        ys = []
        for nb in range(4):
            n = 128 if nb < 3 else 64
            blk = wot_v.at[pl.ds(nb * 128, n)]
            wait_all(blk, wsem.at[WO + nb])
            ys.append(lax.dot_general(ob, blk[...], NT, preferred_element_type=f32))
        y = jnp.concatenate(ys, axis=1) + base
        out_v[0] = y[0:1].astype(bf)
        co = pltpu.make_async_copy(out_v, o_hbm, wsem.at[OUT]); co.start(); co.wait()

    def f(A_x, A_k, A_v, A_wq, A_wo, B_x, B_w1, B_b1, B_w2):
        hbm = pl.BlockSpec(memory_space=pltpu.HBM)
        return pl.pallas_call(
            kernel, out_shape=jax.ShapeDtypeStruct((1, 1, D), bf),
            in_specs=[hbm] * 8, out_specs=hbm,
            scratch_shapes=[
                pltpu.VMEM((1, 1, D), bf), pltpu.VMEM((F // 128, 128), bf),
                pltpu.VMEM((D, H * DH), bf), pltpu.VMEM((D, H * DH), bf),
                pltpu.VMEM((D, F), bf), pltpu.VMEM((D, F), bf),
                pltpu.VMEM((nbuf, H, T, DH), bf), pltpu.VMEM((NG, H, T), f32),
                pltpu.VMEM((H, 8, DH), f32), pltpu.VMEM((8, H * DH), f32), pltpu.VMEM((1, 1, D), bf),
                pltpu.SemaphoreType.DMA((nbuf,)), pltpu.SemaphoreType.DMA((10,))],
            compiler_params=pltpu.CompilerParams(vmem_limit_bytes=64 << 20, disable_bounds_checks=nobc,
                                                 disable_semaphore_checks=nosc),
        )(A_x, A_k, A_v, A_wq, A_wo.T, B_w1, B_b1.reshape(F // 128, 128), B_w2.T)
    return f


@jax.jit
def pallas_parallel_sum__mha_block_cached__dense_activation_mish__decode_kernel(
    A_x, A_k_cache, A_v_cache, A_wq, A_wo, B_x, B_w1, B_b1, B_w2):
    return make(lag=3, nbuf=4)(A_x, A_k_cache, A_v_cache, A_wq, A_wo, B_x, B_w1, B_b1, B_w2)
```

```python
import jax
import jax.numpy as jnp
from jax import lax
from jax.experimental import pallas as pl
from jax.experimental.pallas import tpu as pltpu

BF16, F32 = jnp.bfloat16, jnp.float32
D, H, SK, DH, F = 448, 16, 16384, 256, 1792

ROWS = 128
GROUPS = SK // ROWS
AHEAD, SLOTS = 3, 4
F_TILES = F // 128
WIDE = (D // 8) * 2
NARROW = D * F // 16384
HALF = H * DH // 2
CONTRACT_LAST = (((1,), (1,)), ((), ()))

WO_BLOCKS = ((0, 448, 0), (0, 256, HALF), (256, 128, HALF), (384, 64, HALF))


def _wo_queues():
    order = []
    for b, (row, rows, col) in enumerate(WO_BLOCKS):
        n = rows // 8
        order += [(b, (row // 8 + i * 9 % n) * 2 + col // HALF) for i in range(n)]
    lead = 28
    return (order[:lead] + order[lead:WIDE - lead:2],
            order[lead + 1:WIDE - lead:2] + order[WIDE - lead:])


def _wide_copy(src, dst, piece, sem):
    row, col = (piece >> 1) * 8, (piece & 1) * HALF
    if not isinstance(piece, int):
        row, col = pl.multiple_of(row, 8), pl.multiple_of(col, HALF)
    idx = (pl.ds(row, 8), pl.ds(col, HALF))
    return pltpu.make_async_copy(src.at[idx], dst.at[idx], sem)


def _narrow_copy(src, dst, piece, sem):
    idx = pl.ds(piece * 16, 16)
    return pltpu.make_async_copy(src.at[idx], dst.at[idx], sem)


def _wait_filled(ref, sem):
    pltpu.make_async_copy(ref, ref, sem).wait()


def _untile(ref):
    return jnp.concatenate(
        [jnp.concatenate([ref[r * F_TILES + c] for r in range(D // 8)], axis=0)
         for c in range(F_TILES)], axis=1)


def _kernel(x_hbm, k_hbm, v_hbm, wq_hbm, wot_hbm, w1_hbm, b1_hbm, w2t_hbm, out_hbm,
            x_v, b1_v, wq_v, wot_v, w1_v, w2t_v, ring, scores, q_v, out_v, ring_sems, sems):

    def start_group(cache, g):
        slot = g & (SLOTS - 1)

        def half(i, _):
            off = pl.multiple_of(i * 64, 64)
            src_rows = pl.ds(pl.multiple_of(g * ROWS + off, 64), 64)
            for h in range(H):
                pltpu.make_async_copy(cache.at[0, h, src_rows, :],
                                      ring.at[slot, h, pl.ds(off, 64), :],
                                      ring_sems.at[slot]).start(priority=h % 2)

        lax.fori_loop(0, 2, half, None)

    sem = sems.at[0]
    q_stride, f_stride, f_first = 19, 17, 4
    pairs = 2 * (NARROW - f_first)
    for i in range(WIDE - pairs):
        _wide_copy(wq_hbm, wq_v, i * q_stride % WIDE, sem).start(priority=1)
    for i in range(f_first):
        _narrow_copy(w1_hbm, w1_v, i * f_stride % NARROW, sem).start(priority=1)
        _narrow_copy(w2t_hbm, w2t_v, i * f_stride % NARROW, sem).start(priority=1)

    def start_pair(i, pieces):
        p, f = pieces

        @pl.when((i & 1) == 0)
        def _():
            _narrow_copy(w1_hbm, w1_v, f, sem).start(priority=0)

        @pl.when((i & 1) == 1)
        def _():
            _narrow_copy(w2t_hbm, w2t_v, f, sem).start(priority=0)

        _wide_copy(wq_hbm, wq_v, p, sem).start(priority=1)
        p, f = p + q_stride, f + (i & 1) * f_stride
        return jnp.where(p >= WIDE, p - WIDE, p), jnp.where(f >= NARROW, f - NARROW, f)

    lax.fori_loop(0, pairs, start_pair, (jnp.int32((WIDE - pairs) * q_stride % WIDE),
                                         jnp.int32(f_first * f_stride % NARROW)))
    pltpu.make_async_copy(x_hbm, x_v, sem).start()
    pltpu.make_async_copy(b1_hbm, b1_v, sem).start()
    lax.fori_loop(0, AHEAD, lambda g, _: start_group(k_hbm, g), None)
    for ref in (x_v, b1_v, wq_v, w1_v, w2t_v):
        _wait_filled(ref, sem)

    x = x_v[0].astype(F32)
    centered = x - jnp.mean(x, axis=-1, keepdims=True)
    var = jnp.mean(centered * centered, axis=-1, keepdims=True)
    xn = jnp.broadcast_to(centered / jnp.sqrt(var + 1e-5), (8, D)).astype(BF16)
    sublane = lax.broadcasted_iota(jnp.int32, (8, DH), 0)

    def project_q(a, _):
        for j in range(8):
            h = a * 8 + j
            wq = wq_v[:, pl.ds(pl.multiple_of(h * DH, DH), DH)]
            q = jnp.dot(xn, wq, preferred_element_type=F32) * DH ** -0.5
            q_v[h] = jnp.where(sublane == j, q, 0.0)

    lax.fori_loop(0, 2, project_q, None)

    def k_step(g, running_max):
        @pl.when(g + AHEAD < GROUPS)
        def _():
            start_group(k_hbm, g + AHEAD)

        @pl.when(g + AHEAD >= GROUPS)
        def _():
            start_group(v_hbm, g + AHEAD - GROUPS)

        slot = g & (SLOTS - 1)
        _wait_filled(ring.at[slot], ring_sems.at[slot])
        s = [lax.dot_general(q_v[h].astype(BF16), ring[slot, h], CONTRACT_LAST,
                             preferred_element_type=F32) for h in range(H)]
        s = jnp.concatenate([sum(s[1:8], s[0]), sum(s[9:], s[8])], axis=0)
        scores[g] = s
        return jnp.maximum(running_max, s)

    row_max = lax.fori_loop(0, GROUPS, k_step, jnp.full((H, ROWS), -jnp.inf, F32))
    row_max = jnp.broadcast_to(jnp.max(row_max, axis=-1, keepdims=True), (H, ROWS))

    b1 = b1_v[...].astype(F32)
    bias = jnp.concatenate(
        [jnp.broadcast_to(b1[c:c + 1], (8, 128)) for c in range(F_TILES)], axis=1)
    hidden = jnp.dot(xn, _untile(w1_v), preferred_element_type=F32) + bias
    softplus = jnp.log1p(jnp.exp(-jnp.abs(hidden))) + jnp.maximum(hidden, 0.0)
    act = (hidden * jnp.tanh(softplus)).astype(BF16)
    y = lax.dot_general(act, _untile(w2t_v), CONTRACT_LAST, preferred_element_type=F32) + x

    wo_queues = _wo_queues()
    wo_pairs = WIDE // 2

    def v_step(g, carry):
        denom, *acc = carry

        @pl.when(g + AHEAD < GROUPS)
        def _():
            start_group(v_hbm, g + AHEAD)

        for part in range(AHEAD):
            @pl.when(g + AHEAD == GROUPS + part)
            def _():
                for i in range(part * wo_pairs // AHEAD, (part + 1) * wo_pairs // AHEAD):
                    for priority, queue in enumerate(wo_queues):
                        block, piece = queue[i]
                        _wide_copy(wot_hbm, wot_v, piece, sems.at[block]).start(priority=priority)

        slot = g & (SLOTS - 1)
        _wait_filled(ring.at[slot], ring_sems.at[slot])
        p = jnp.exp(scores[g] - row_max)
        for h in range(H):
            a = h // 8
            p_head = jnp.where(sublane[:, :ROWS] == h % 8, p[a * 8:a * 8 + 8], 0.0).astype(BF16)
            acc[a] = acc[a] + jnp.dot(p_head, ring[slot, h], preferred_element_type=F32)
        return (denom + p, *acc)

    zeros = jnp.zeros((8, DH), F32)
    denom, *acc = lax.fori_loop(0, GROUPS, v_step, (jnp.zeros((H, ROWS), F32), zeros, zeros))
    o = jnp.concatenate(acc, axis=0) / jnp.sum(denom, axis=-1, keepdims=True)
    o = jnp.concatenate(
        [jnp.broadcast_to(o[h:h + 1], (8, DH)) for h in range(H)], axis=1).astype(BF16)

    for block, (row, rows, col) in enumerate(WO_BLOCKS):
        wot = wot_v.at[pl.ds(row, rows), pl.ds(col, HALF)]
        _wait_filled(wot, sems.at[block])
        part = lax.dot_general(o[:, col:col + HALF], wot[...], CONTRACT_LAST,
                               preferred_element_type=F32)
        padded = [part]
        if row:
            padded.insert(0, jnp.zeros((8, row), F32))
        if row + rows < D:
            padded.append(jnp.zeros((8, D - row - rows), F32))
        y = y + jnp.concatenate(padded, axis=1)

    out_v[0] = y[0:1].astype(BF16)
    store = pltpu.make_async_copy(out_v, out_hbm, sem)
    store.start()
    store.wait()


def _as_tiles(w):
    rows, cols = w.shape
    w = w.reshape(rows // 8, 8, cols // 128, 128).transpose(0, 2, 1, 3)
    return w.reshape(rows // 8 * (cols // 128), 8, 128)


@jax.jit
def pallas_parallel_sum__mha_block_cached__dense_activation_mish__decode_kernel(
    A_x: jax.Array,
    A_k_cache: jax.Array,
    A_v_cache: jax.Array,
    A_wq: jax.Array,
    A_wo: jax.Array,
    B_x: jax.Array,
    B_w1: jax.Array,
    B_b1: jax.Array,
    B_w2: jax.Array,
):
    del B_x
    hbm = pl.BlockSpec(memory_space=pltpu.HBM)
    ffn_tiles = (D // 8 * F_TILES, 8, 128)
    return pl.pallas_call(
        _kernel,
        out_shape=jax.ShapeDtypeStruct((1, 1, D), BF16),
        in_specs=[hbm] * 8,
        out_specs=hbm,
        scratch_shapes=[
            pltpu.VMEM((1, 1, D), BF16),
            pltpu.VMEM((F_TILES, 128), BF16),
            pltpu.VMEM((D, H * DH), BF16),
            pltpu.VMEM((D, H * DH), BF16),
            pltpu.VMEM(ffn_tiles, BF16),
            pltpu.VMEM(ffn_tiles, BF16),
            pltpu.VMEM((SLOTS, H, ROWS, DH), BF16),
            pltpu.VMEM((GROUPS, H, ROWS), F32),
            pltpu.VMEM((H, 8, DH), F32),
            pltpu.VMEM((1, 1, D), BF16),
            pltpu.SemaphoreType.DMA((SLOTS,)),
            pltpu.SemaphoreType.DMA((len(WO_BLOCKS),)),
        ],
        compiler_params=pltpu.CompilerParams(
            vmem_limit_bytes=48 << 20, disable_semaphore_checks=True),
    )(A_x, A_k_cache, A_v_cache, A_wq, A_wo.T, _as_tiles(B_w1),
      B_b1.reshape(F_TILES, 128), _as_tiles(B_w2.T))
```

```python
import jax
import jax.numpy as jnp
from jax import lax
from jax.experimental import pallas as pl
from jax.experimental.pallas import tpu as pltpu

BF16, F32 = jnp.bfloat16, jnp.float32
D, H, SK, DH, F = 448, 16, 16384, 256, 1792

ROWS = 128
GROUPS = SK // ROWS
AHEAD, SLOTS = 3, 4
F_TILES = F // 128
WIDE = (D // 8) * 2
NARROW = D * F // 16384
HALF = H * DH // 2
CONTRACT_LAST = (((1,), (1,)), ((), ()))

WO_BLOCKS = ((0, 448, 0, 9), (0, 256, HALF, 17), (256, 128, HALF, 9), (384, 64, HALF, 1))


def _wo_batches():
    order = []
    for block, (row, rows, col, stride) in enumerate(WO_BLOCKS):
        n = rows // 8
        order += [(block, (row // 8 + i * stride % n) * 2 + col // HALF) for i in range(n)]
    lead = 28
    pairs = list(zip(order[:lead] + order[lead:WIDE - lead:2],
                     order[lead + 1:WIDE - lead:2] + order[WIDE - lead:], strict=True))
    return [[pair for pair in pairs if max(pair)[0] == b] for b in range(len(WO_BLOCKS))]


def _wide_copy(src, dst, piece, sem):
    row, col = (piece >> 1) * 8, (piece & 1) * HALF
    if not isinstance(piece, int):
        row, col = pl.multiple_of(row, 8), pl.multiple_of(col, HALF)
    idx = (pl.ds(row, 8), pl.ds(col, HALF))
    return pltpu.make_async_copy(src.at[idx], dst.at[idx], sem)


def _narrow_copy(src, dst, piece, sem):
    idx = pl.ds(piece * 16, 16)
    return pltpu.make_async_copy(src.at[idx], dst.at[idx], sem)


def _wait_filled(ref, sem):
    pltpu.make_async_copy(ref, ref, sem).wait()


def _untile(ref):
    return jnp.concatenate(
        [jnp.concatenate([ref[r * F_TILES + c] for r in range(D // 8)], axis=0)
         for c in range(F_TILES)], axis=1)


def _kernel(x_hbm, k_hbm, v_hbm, wq_hbm, wot_hbm, w1_hbm, b1_hbm, w2t_hbm, out_hbm,
            x_v, b1_v, wq_v, wot_v, w1_v, w2t_v, ring, scores, q_v, out_v, sems):

    def start_group(cache, g):
        slot = g & (SLOTS - 1)

        def half(i, _):
            off = pl.multiple_of(i * 64, 64)
            src_rows = pl.ds(pl.multiple_of(g * ROWS + off, 64), 64)
            for h in range(H):
                pltpu.make_async_copy(cache.at[0, h, src_rows, :],
                                      ring.at[slot, h, pl.ds(off, 64), :],
                                      sems.at[slot]).start(priority=h % 2)

        lax.fori_loop(0, 2, half, None)

    sem = sems.at[SLOTS - 1]
    q_stride, f_first = 45, 4
    pairs = 2 * (NARROW - f_first)
    for i in range(WIDE - pairs):
        _wide_copy(wq_hbm, wq_v, i * q_stride % WIDE, sem).start(priority=1)
    for i in range(f_first):
        _narrow_copy(w1_hbm, w1_v, i, sem).start(priority=1)
        _narrow_copy(w2t_hbm, w2t_v, i, sem).start(priority=1)

    def start_pair(i, piece):
        @pl.when((i & 1) == 0)
        def _():
            _narrow_copy(w1_hbm, w1_v, f_first + (i >> 1), sem).start(priority=0)

        @pl.when((i & 1) == 1)
        def _():
            _narrow_copy(w2t_hbm, w2t_v, f_first + (i >> 1), sem).start(priority=0)

        _wide_copy(wq_hbm, wq_v, piece, sem).start(priority=1)
        piece = piece + q_stride
        return jnp.where(piece >= WIDE, piece - WIDE, piece)

    lax.fori_loop(0, pairs, start_pair, jnp.int32((WIDE - pairs) * q_stride % WIDE))
    pltpu.make_async_copy(x_hbm, x_v, sem).start()
    pltpu.make_async_copy(b1_hbm, b1_v, sem).start()
    lax.fori_loop(0, AHEAD, lambda g, _: start_group(k_hbm, g), None)
    for ref in (x_v, b1_v, wq_v, w1_v, w2t_v):
        _wait_filled(ref, sem)

    x = x_v[0].astype(F32)
    centered = x - jnp.mean(x, axis=-1, keepdims=True)
    var = jnp.mean(centered * centered, axis=-1, keepdims=True)
    xn = jnp.broadcast_to(centered / jnp.sqrt(var + 1e-5), (8, D)).astype(BF16)
    sublane = lax.broadcasted_iota(jnp.int32, (8, DH), 0)

    def project_q(a, _):
        for j in range(8):
            h = a * 8 + j
            wq = wq_v[:, pl.ds(pl.multiple_of(h * DH, DH), DH)]
            q = jnp.dot(xn, wq, preferred_element_type=F32) * DH ** -0.5
            q_v[h] = jnp.where(sublane == j, q, 0.0)

    lax.fori_loop(0, 2, project_q, None)

    def k_step(g, running_max):
        @pl.when(g + AHEAD < GROUPS)
        def _():
            start_group(k_hbm, g + AHEAD)

        @pl.when(g + AHEAD >= GROUPS)
        def _():
            start_group(v_hbm, g + AHEAD - GROUPS)

        slot = g & (SLOTS - 1)
        _wait_filled(ring.at[slot], sems.at[slot])
        s = [lax.dot_general(q_v[h].astype(BF16), ring[slot, h], CONTRACT_LAST,
                             preferred_element_type=F32) for h in range(H)]
        s = jnp.concatenate([sum(s[1:8], s[0]), sum(s[9:], s[8])], axis=0)
        scores[g] = s
        return jnp.maximum(running_max, s)

    row_max = lax.fori_loop(0, GROUPS, k_step, jnp.full((H, ROWS), -jnp.inf, F32))
    row_max = jnp.broadcast_to(jnp.max(row_max, axis=-1, keepdims=True), (H, ROWS))

    b1 = b1_v[...].astype(F32)
    bias = jnp.concatenate(
        [jnp.broadcast_to(b1[c:c + 1], (8, 128)) for c in range(F_TILES)], axis=1)
    hidden = jnp.dot(xn, _untile(w1_v), preferred_element_type=F32) + bias
    softplus = jnp.log1p(jnp.exp(-jnp.abs(hidden))) + jnp.maximum(hidden, 0.0)
    act = (hidden * jnp.tanh(softplus)).astype(BF16)
    y = lax.dot_general(act, _untile(w2t_v), CONTRACT_LAST, preferred_element_type=F32) + x

    def start_wo(batch):
        for pair in _wo_batches()[batch]:
            for priority, (block, piece) in enumerate(pair):
                _wide_copy(wot_hbm, wot_v, piece, sems.at[block]).start(priority=priority)

    def v_step(g, carry):
        denom, *acc = carry

        @pl.when(g + AHEAD < GROUPS)
        def _():
            start_group(v_hbm, g + AHEAD)

        for batch in range(AHEAD):
            @pl.when(g + AHEAD == GROUPS + batch)
            def _():
                start_wo(batch)

        slot = g & (SLOTS - 1)
        _wait_filled(ring.at[slot], sems.at[slot])
        p = jnp.exp(scores[g] - row_max)
        for h in range(H):
            a = h // 8
            p_head = jnp.where(sublane[:, :ROWS] == h % 8, p[a * 8:a * 8 + 8], 0.0).astype(BF16)
            acc[a] = acc[a] + jnp.dot(p_head, ring[slot, h], preferred_element_type=F32)
        return (denom + p, *acc)

    zeros = jnp.zeros((8, DH), F32)
    denom, *acc = lax.fori_loop(0, GROUPS, v_step, (jnp.zeros((H, ROWS), F32), zeros, zeros))
    start_wo(AHEAD)
    o = jnp.concatenate(acc, axis=0) / jnp.sum(denom, axis=-1, keepdims=True)
    o = jnp.concatenate(
        [jnp.broadcast_to(o[h:h + 1], (8, DH)) for h in range(H)], axis=1).astype(BF16)

    for block, (row, rows, col, _) in enumerate(WO_BLOCKS):
        wot = wot_v.at[pl.ds(row, rows), pl.ds(col, HALF)]
        _wait_filled(wot, sems.at[block])
        part = lax.dot_general(o[:, col:col + HALF], wot[...], CONTRACT_LAST,
                               preferred_element_type=F32)
        padded = [part]
        if row:
            padded.insert(0, jnp.zeros((8, row), F32))
        if row + rows < D:
            padded.append(jnp.zeros((8, D - row - rows), F32))
        y = y + jnp.concatenate(padded, axis=1)

    out_v[0] = y[0:1].astype(BF16)
    store = pltpu.make_async_copy(out_v, out_hbm, sem)
    store.start()
    store.wait()


def _as_tiles(w):
    rows, cols = w.shape
    w = w.reshape(rows // 8, 8, cols // 128, 128).transpose(0, 2, 1, 3)
    return w.reshape(rows // 8 * (cols // 128), 8, 128)


@jax.jit
def pallas_parallel_sum__mha_block_cached__dense_activation_mish__decode_kernel(
    A_x: jax.Array,
    A_k_cache: jax.Array,
    A_v_cache: jax.Array,
    A_wq: jax.Array,
    A_wo: jax.Array,
    B_x: jax.Array,
    B_w1: jax.Array,
    B_b1: jax.Array,
    B_w2: jax.Array,
):
    del B_x
    hbm = pl.BlockSpec(memory_space=pltpu.HBM)
    ffn_tiles = (D // 8 * F_TILES, 8, 128)
    return pl.pallas_call(
        _kernel,
        out_shape=jax.ShapeDtypeStruct((1, 1, D), BF16),
        in_specs=[hbm] * 8,
        out_specs=hbm,
        scratch_shapes=[
            pltpu.VMEM((1, 1, D), BF16),
            pltpu.VMEM((F_TILES, 128), BF16),
            pltpu.VMEM((D, H * DH), BF16),
            pltpu.VMEM((D, H * DH), BF16),
            pltpu.VMEM(ffn_tiles, BF16),
            pltpu.VMEM(ffn_tiles, BF16),
            pltpu.VMEM((SLOTS, H, ROWS, DH), BF16),
            pltpu.VMEM((GROUPS, H, ROWS), F32),
            pltpu.VMEM((H, 8, DH), F32),
            pltpu.VMEM((1, 1, D), BF16),
            pltpu.SemaphoreType.DMA((SLOTS,)),
        ],
        compiler_params=pltpu.CompilerParams(vmem_limit_bytes=48 << 20),
    )(A_x, A_k_cache, A_v_cache, A_wq, A_wo.T, _as_tiles(B_w1),
      B_b1.reshape(F_TILES, 128), _as_tiles(B_w2.T))
```
